```python
import os as _os
_os.environ.setdefault("JAX_PLATFORMS", "cpu")
import jax
import jax.numpy as jnp

def _softmax(x, axis=-1):
    return jax.nn.softmax(x, axis=axis)
def _gelu(x):
    return jax.nn.gelu(x, approximate=True)
def _silu(x):
    return jax.nn.silu(x)
def _sigmoid(x):
    return jax.nn.sigmoid(x)
def _layernorm(x, axis=-1, eps=1e-5):
    m = jnp.mean(x, axis=axis, keepdims=True)
    v = jnp.var(x, axis=axis, keepdims=True)
    return (x - m) / jnp.sqrt(v + eps)
def _scatter_add(tgt, idx, src, axis=0):
    return tgt.at[idx].add(src)
def _segment_sum(src, seg, n):
    return jax.ops.segment_sum(src, seg, n)
class _Rng:
    def __init__(self, key):
        self._k = key
    def _next(self):
        self._k, sub = jax.random.split(self._k)
        return sub
    def normal(self, shape):
        return jax.random.normal(self._next(), shape, dtype=jnp.bfloat16)
    def randint(self, lo, hi, shape):
        return jax.random.randint(self._next(), shape, lo, hi, dtype=jnp.int32)
    def uniform(self, shape, lo=0.0, hi=1.0):
        return jax.random.uniform(self._next(), shape, jnp.bfloat16, lo, hi)
    def permutation(self, n):
        return jax.random.permutation(self._next(), n)


kernel_name = 'concat_heads__gqa_block_cached__gqa_block_cached__near_ridge'

def setup_inputs():
    _rng = _Rng(jax.random.key(int.from_bytes(__import__("os").urandom(4), "little")))
    _w = (lambda a: (lambda t: t.astype(jnp.bfloat16) if jnp.issubdtype(t.dtype, jnp.floating) else t)(jnp.asarray(a)))
    def _A_setup():
        B, Sq, D = 8, 240, 640
        Hq, Hkv, Sk, Dh = 32, 32, 1024, 192
        assert Hq % Hkv == 0, (Hq, Hkv)
        return {
            "x": _w((lambda *s: _rng.normal(s) * 0.8)(B, Sq, D)),
            "k_cache": _w((lambda *s: _rng.normal(s) * 0.8)(B, Hkv, Sk, Dh)),
            "v_cache": _w((lambda *s: _rng.normal(s) * 0.05)(B, Hkv, Sk, Dh)),
            "wq": _w((lambda *s: _rng.normal(s) * 0.8)(D, Hq * Dh) * (D ** -0.5)),
            "wo": _w((lambda *s: _rng.normal(s) * 0.05)(Hq * Dh, D) * ((Hq * Dh) ** -0.5)),
        }
    _A_in = _A_setup()

    def _B_setup():
        B, Sq, D = 8, 240, 640
        Hq, Hkv, Sk, Dh = 32, 32, 1024, 192
        assert Hq % Hkv == 0, (Hq, Hkv)
        return {
            "x": _w((lambda *s: _rng.normal(s) * 0.8)(B, Sq, D)),
            "k_cache": _w((lambda *s: _rng.normal(s) * 0.8)(B, Hkv, Sk, Dh)),
            "v_cache": _w((lambda *s: _rng.normal(s) * 0.05)(B, Hkv, Sk, Dh)),
            "wq": _w((lambda *s: _rng.normal(s) * 0.8)(D, Hq * Dh) * (D ** -0.5)),
            "wo": _w((lambda *s: _rng.normal(s) * 0.05)(Hq * Dh, D) * ((Hq * Dh) ** -0.5)),
        }
    _B_in = _B_setup()

    return {
        "A_x": _A_in["x"],
        "A_k_cache": _A_in["k_cache"],
        "A_v_cache": _A_in["v_cache"],
        "A_wq": _A_in["wq"],
        "A_wo": _A_in["wo"],
        "B_x": _B_in["x"],
        "B_k_cache": _B_in["k_cache"],
        "B_v_cache": _B_in["v_cache"],
        "B_wq": _B_in["wq"],
        "B_wo": _B_in["wo"],
    }

def reference(A_x, A_k_cache, A_v_cache, A_wq, A_wo, B_x, B_k_cache, B_v_cache, B_wq, B_wo):
    def _A_ref(x, k_cache, v_cache, wq, wo):
        B, Sq, D = x.shape
        Hq, Dh = 32, 192
        Hkv = k_cache.shape[1]
        rep = Hq // Hkv
        q = (lambda x, *d: x.transpose(*d))((x @ wq).reshape(B, Sq, Hq, Dh), 0, 2, 1, 3)
        k = jnp.repeat(k_cache, rep, axis=1)
        v = jnp.repeat(v_cache, rep, axis=1)
        scores = jnp.einsum("bhqd,bhkd->bhqk", q, k) * (Dh ** -0.5)
        p = _softmax(scores, axis=-1)
        o = jnp.einsum("bhqk,bhkd->bhqd", p, v)
        return (lambda x, *d: x.transpose(*d))(o, 0, 2, 1, 3).reshape(B, Sq, Hq * Dh) @ wo

    def _B_ref(x, k_cache, v_cache, wq, wo):
        B, Sq, D = x.shape
        Hq, Dh = 32, 192
        Hkv = k_cache.shape[1]
        rep = Hq // Hkv
        q = (lambda x, *d: x.transpose(*d))((x @ wq).reshape(B, Sq, Hq, Dh), 0, 2, 1, 3)
        k = jnp.repeat(k_cache, rep, axis=1)
        v = jnp.repeat(v_cache, rep, axis=1)
        scores = jnp.einsum("bhqd,bhkd->bhqk", q, k) * (Dh ** -0.5)
        p = _softmax(scores, axis=-1)
        o = jnp.einsum("bhqk,bhkd->bhqd", p, v)
        return (lambda x, *d: x.transpose(*d))(o, 0, 2, 1, 3).reshape(B, Sq, Hq * Dh) @ wo

    a = _A_ref(A_x, A_k_cache, A_v_cache, A_wq, A_wo)
    b = _B_ref(B_x, B_k_cache, B_v_cache, B_wq, B_wo)
    return jnp.concatenate([a, b], axis=-1)
```

```python
import numpy as np
import jax
import jax.numpy as jnp
from jax import lax
import jax.experimental.pallas as pl
import jax.experimental.pallas.tpu as pltpu

B, SQ, D = 8, 240, 640
H, SK, DH = 32, 1024, 192
PW = 2 * DH
NP = H // 2
T = NP * B
R = 4
T1 = 4
RG = 16
QT = ((0, 128), (128, SQ))
LOG2E = 1.4426950408889634
F32, BF16 = jnp.float32, jnp.bfloat16
NT = (((1,), (1,)), ((), ()))

ORDER_FINE = 'q0-q1-q2-k00-k01-k02-k03-k04-k05-k06-k07-k10-k11-k12-k13-k14-k15-k16-k17-P00-P01-P10-t0-P11-t1-o0-o1-o2-o3-o4'
ORDER_U1 = 'q0-q1-q2-k00-k01-k02-k03-k04-k05-k06-k07-k10-k11-P00-P01-P10-t0-P11-t1-k12-k13-k14-k15-k16-o0-o1-o2-o3-o4-k17'
ORDER_LAST = ORDER_U1
ORD4 = [
    'q0-q1-q2-k02-k03-k00-k01-k04-k05-k06-k07-k10-k11-P00-P01-P11-P10-t0-t1-k14-k12-k13-k15-k16-o0-o1-o2-o3-o4-k17',
    'q0-q1-q2-k00-k02-k03-k04-k05-k01-k06-k07-k11-k10-P00-P01-P10-t0-k16-P11-t1-k14-k15-k13-k12-o0-o1-o2-o4-k17-o3',
    'q0-q1-q2-k00-k01-k02-k03-k04-k06-k07-k10-k11-P00-k05-P01-P10-t0-P11-t1-k12-k13-k16-k14-o1-k15-o0-o2-o3-o4-k17',
    'q0-q1-k00-q2-k01-k02-k03-k04-k05-k06-k07-k10-k11-P00-P01-P10-t0-P11-t1-k12-k13-k14-k15-o0-k16-o2-o1-o3-o4-k17',
]
HOOK = 12
HOOK1 = 3
SEARCH = 0


def _qk_tasks(x_ref, wq_ref, kt_ref, q_scr, s_scr):
    c = np.float32(DH ** -0.5 * LOG2E)

    def qproj(n):
        def f():
            q = jnp.dot(x_ref[...], wq_ref[:, n * 128:(n + 1) * 128], preferred_element_type=F32) * c
            if n == 0:
                q_scr[0] = q.astype(BF16)
            elif n == 2:
                q_scr[3] = q.astype(BF16)
            else:
                lane = lax.broadcasted_iota(jnp.int32, (SQ, 128), 1)
                q_scr[1] = jnp.where(lane < 64, q, 0.0).astype(BF16)
                q_scr[2] = jnp.where(lane >= 64, q, 0.0).astype(BF16)
        return f

    def qk(hh, n):
        def f():
            qq = jnp.concatenate([q_scr[2 * hh], q_scr[2 * hh + 1]], axis=1)
            s_scr[hh, :, n * 128:(n + 1) * 128] = jnp.dot(
                qq, kt_ref[hh * 128:hh * 128 + 256, n * 128:(n + 1) * 128], preferred_element_type=F32)
        return f

    tasks = {'q%d' % n: qproj(n) for n in range(3)}
    tasks.update({'k%d%d' % (hh, n): qk(hh, n) for hh in range(2) for n in range(8)})
    return tasks


def _softmax(s_scr, p_scr, l_scr):
    for hh in range(2):
        for r in range(SQ // RG):
            rows = slice(r * RG, (r + 1) * RG)
            s = s_scr[hh, rows, :]
            m = jnp.broadcast_to(jnp.max(s, axis=-1, keepdims=True), (RG, 128))
            acc = None
            for n in range(8):
                e = jnp.exp2(s[:, n * 128:(n + 1) * 128] - m)
                p_scr[hh, n, rows, :] = e.astype(BF16)
                acc = e if acc is None else acc + e
            l_scr[hh, rows, :] = acc


def _pv_tasks(vt_ref, wo_ref, p_scr, l_scr, ot_scr, o_scr, acc_ref, st_ref):
    def pv(hh, qt):
        lo, hi = QT[qt]

        def f():
            p = jnp.concatenate([p_scr[hh, n, lo:hi, :] for n in range(8)], axis=1)
            ot = lax.dot_general(vt_ref[hh * DH:(hh + 1) * DH, :], p, NT, preferred_element_type=F32)
            l = jnp.sum(l_scr[hh, lo:hi, :].T, axis=0, keepdims=True)
            ot_scr[qt, hh * DH:(hh + 1) * DH, 0:hi - lo] = (ot * (1.0 / l)).astype(BF16)
        return f

    def tr(qt):
        lo, hi = QT[qt]

        def f():
            for kt in range(3):
                o_scr[kt, lo:hi, :] = ot_scr[qt, kt * 128:(kt + 1) * 128, 0:hi - lo].T
        return f

    def outp(n):
        def f():
            cols = slice(n * 128, (n + 1) * 128)
            o = jnp.concatenate([o_scr[0], o_scr[1], o_scr[2]], axis=1)
            new = acc_ref[:, cols] + jnp.dot(o, wo_ref[:, cols], preferred_element_type=F32)
            acc_ref[:, cols] = new
            st_ref[:, cols] = new.astype(BF16)
        return f

    tasks = {'P%d%d' % (hh, qt): pv(hh, qt) for hh in range(2) for qt in range(2)}
    tasks.update({'t%d' % qt: tr(qt) for qt in range(2)})
    tasks.update({'o%d' % n: outp(n) for n in range(5)})
    return tasks


def _sub(order, qk_args, sm_args, pv_args, pre=None, hook=None, hook_pos=0):
    pre = dict(pre or {})
    tasks = {}
    if qk_args:
        tasks.update(_qk_tasks(*qk_args))
    if pv_args:
        tasks.update(_pv_tasks(*pv_args))
    if 'q' in pre:
        pre.pop('q')()
    if sm_args:
        _softmax(*sm_args)
    idx = 0
    for name in order.split('-'):
        if name not in tasks:
            continue
        if hook is not None and idx == hook_pos:
            hook()
            hook = None
        if name[0] in pre:
            pre.pop(name[0])()
        tasks[name]()
        idx += 1
    assert hook is None and not pre


def _kernel(xa_h, kta_h, vta_h, wqa_h, woa_h, xb_h, ktb_h, vtb_h, wqb_h, wob_h, out_h,
            xr, kvr, wqa, wqb, woa, wob, acc_a, acc_b,
            qa, qb, sa, sb, pa, pb, la, lb, ota, otb, oa, ob, ostage,
            sem, sem_p, sem_o):
    XB, XA, KB, VA, KA, VB = 0, 1, 0, 1, 2, 3

    def slot(t):
        return (t + 1) & (R - 1)

    def kv_src(h, t):
        tc = jnp.minimum(t, T - 1)
        return h.at[tc & 7, pl.ds(pl.multiple_of((tc >> 3) * PW, 128), PW), :]

    def w_region(dst, c, n, is_q):
        g1 = jnp.minimum((c >> 3) + 1, NP)
        if is_q:
            return dst.at[g1, pl.ds(pl.multiple_of((c & 7) * 80, 16), 80 * n), :]
        return dst.at[g1, pl.ds(pl.multiple_of((c & 7) * 48, 16), 48 * n), :]

    def w_src(h, c, is_q):
        gc = jnp.minimum((c >> 3) + 1, NP - 1)
        if is_q:
            return h.at[pl.ds(pl.multiple_of((c & 7) * 80, 16), 80), pl.ds(pl.multiple_of(gc * PW, 128), PW)]
        return h.at[pl.ds(pl.multiple_of(gc * PW + (c & 7) * 48, 16), 48), :]

    def blocks(t, steady):
        sl = slot(t)

        def cp(src, dst, half, kind):
            fine, coarse = sl * 2 + half, 2 * R + (sl >> 1) * 6 + kind
            idx = coarse if steady else jnp.where(t <= T1, fine, coarse)
            return pltpu.make_async_copy(src, dst, sem.at[idx])
        return ([cp(xb_h.at[t & 7], xr.at[sl, XB], 0, 1),
                 cp(kv_src(ktb_h, t), kvr.at[sl, KB], 0, 0),
                 cp(kv_src(vta_h, t), kvr.at[sl, VA], 0, 0),
                 cp(w_src(wqb_h, t - 1, True), w_region(wqb, t - 1, 1, True), 0, 3),
                 cp(w_src(woa_h, t - 1, False), w_region(woa, t - 1, 1, False), 0, 4)],
                [cp(xa_h.at[(t + 1) & 7], xr.at[sl, XA], 1, 1),
                 cp(kv_src(kta_h, t + 1), kvr.at[sl, KA], 1, 0),
                 cp(kv_src(vtb_h, t), kvr.at[sl, VB], 1, 0),
                 cp(w_src(wqa_h, t + 1, True), w_region(wqa, t + 1, 1, True), 1, 2),
                 cp(w_src(wob_h, t - 1, False), w_region(wob, t - 1, 1, False), 1, 5)])

    def start_blocks(t, steady):
        h0, h1 = blocks(t, steady)
        for c in h0 + h1:
            c.start()

    def wait_pair(t):
        s0 = pl.multiple_of(slot(t), 2)
        base = 2 * R + (s0 >> 1) * 6
        for kind, region in enumerate((kvr.at[pl.ds(s0, 2)], xr.at[pl.ds(s0, 2)],
                                       w_region(wqa, t + 1, 2, True), w_region(wqb, t - 1, 2, True),
                                       w_region(woa, t - 1, 2, False), w_region(wob, t - 1, 2, False))):
            pltpu.make_async_copy(region, region, sem.at[base + kind]).wait()

    def out_copy(b):
        return pltpu.make_async_copy(ostage.at[b], out_h.at[b], sem_o.at[b])

    def body(j, order1, order2, pre1=None, pre2=None, hook=None, hook_pos=0, last=False, mid=None):
        g, b = j >> 3, j & 7
        gn = (j + 1) >> 3
        sl = slot(j)
        _sub(order1, (xr.at[sl, XB], wqb.at[g], kvr.at[sl, KB], qb, sb), (sa, pa, la),
             (kvr.at[sl, VA], woa.at[g], pa, la, ota, oa, acc_a.at[b], ostage.at[b, :, pl.ds(0, D)]),
             pre1, hook, hook_pos)
        if mid is not None:
            mid()
        _sub(order2, None if last else (xr.at[sl, XA], wqa.at[gn], kvr.at[sl, KA], qa, sa), (sb, pb, lb),
             (kvr.at[sl, VB], wob.at[g], pb, lb, otb, ob, acc_b.at[b], ostage.at[b, :, pl.ds(D, D)]),
             pre2)

    n_p = [0]

    def pc(src, dst):
        n_p[0] += 1
        return pltpu.make_async_copy(src, dst, sem_p.at[n_p[0] - 1])
    first = pl.ds(0, PW)
    p_xa0, p_wqa, p_ka0 = pc(xa_h.at[0], xr.at[0, XA]), pc(wqa_h.at[:, first], wqa.at[0]), pc(kta_h.at[0, first, :], kvr.at[0, KA])
    p_xb0, p_wqb, p_kb0 = pc(xb_h.at[0], xr.at[1, XB]), pc(wqb_h.at[:, first], wqb.at[0]), pc(ktb_h.at[0, first, :], kvr.at[1, KB])
    p_va0, p_woa = pc(vta_h.at[0, first, :], kvr.at[1, VA]), pc(woa_h.at[first, :], woa.at[0])
    p_xa1, p_ka1 = pc(xa_h.at[1], xr.at[1, XA]), pc(kta_h.at[1, first, :], kvr.at[1, KA])
    p_vb0, p_wob = pc(vtb_h.at[0, first, :], kvr.at[1, VB]), pc(wob_h.at[first, :], wob.at[0])
    p_wc0 = pc(w_src(wqa_h, 0, True), w_region(wqa, 0, 1, True))
    p_wc1 = pc(w_src(wqa_h, 1, True), w_region(wqa, 1, 1, True))
    for c in (p_xa0, p_wqa, p_ka0, p_xb0, p_wqb, p_kb0, p_va0, p_woa, p_xa1, p_ka1, p_vb0, p_wob, p_wc0, p_wc1):
        c.start()
    start_blocks(1, False)
    acc_a[...] = jnp.zeros(acc_a.shape, F32)
    acc_b[...] = jnp.zeros(acc_b.shape, F32)

    def waits(*cs):
        def f():
            for c in cs:
                c.wait()
        return f

    if not SEARCH:
        _sub(ORDER_FINE, (xr.at[0, XA], wqa.at[0], kvr.at[0, KA], qa, sa), None, None,
             {'q': waits(p_xa0, p_wqa), 'k': waits(p_ka0)})
        body(0, ORDER_FINE, ORDER_FINE,
             {'q': waits(p_xb0, p_wqb), 'k': waits(p_kb0), 'P': waits(p_va0, p_woa)},
             {'q': waits(p_xa1, p_ka1), 'P': waits(p_vb0, p_wob)},
             lambda: start_blocks(2, False), HOOK1)
        p_wc0.wait()
        p_wc1.wait()

        def body1(j, carry):
            h0, h1 = blocks(j, False)
            body(j, ORDER_U1, ORDER_U1, {'q': waits(*h0)}, {'q': waits(*h1)},
                 lambda: start_blocks(j + 2, False), HOOK1)
            return carry
        lax.fori_loop(1, T1 + 1, body1, 0)

    def body2(i, carry):
        j = T1 + 1 + 2 * i

        def start_next():
            start_blocks(j + 2, True)
            start_blocks(j + 3, True)
        wait_pair(j)
        for k in range(2):
            body(j + k, ORD4[2 * k], ORD4[2 * k + 1], hook=start_next if k == 0 else None, hook_pos=HOOK)
            pl.when(j + k >= T - B)(lambda: out_copy((j + k) & 7).start())
        return carry
    lax.fori_loop(0, (T - 2 - T1) // 2, body2, 0)

    wait_pair(T - 1)
    out_a = pltpu.make_async_copy(ostage.at[B - 1, :, pl.ds(0, D)], out_h.at[B - 1, :, pl.ds(0, D)], sem_o.at[B - 1])
    out_b = pltpu.make_async_copy(ostage.at[B - 1, :, pl.ds(D, D)], out_h.at[B - 1, :, pl.ds(D, D)], sem_o.at[B])
    if not SEARCH:
        body(T - 1, ORDER_LAST, ORDER_LAST, last=True, mid=lambda: out_a.start())
    else:
        out_a.start()
    out_b.start()
    for b in range(B - 1):
        out_copy(b).wait()
    out_a.wait()
    out_b.wait()


@jax.jit
def pallas_concat_heads__gqa_block_cached__gqa_block_cached__near_ridge_kernel(
        A_x, A_k_cache, A_v_cache, A_wq, A_wo, B_x, B_k_cache, B_v_cache, B_wq, B_wo):
    def tr(c):
        return jnp.swapaxes(c, 2, 3).reshape(B, H * DH, SK)
    anyspec = pl.BlockSpec(memory_space=pl.ANY)
    vmem, dma = pltpu.VMEM, pltpu.SemaphoreType.DMA
    return pl.pallas_call(
        _kernel,
        in_specs=[anyspec] * 10,
        out_specs=anyspec,
        out_shape=jax.ShapeDtypeStruct((B, SQ, 2 * D), BF16),
        scratch_shapes=[vmem((R, 2, SQ, D), BF16), vmem((R, 4, PW, SK), BF16),
                        vmem((NP + 1, D, PW), BF16), vmem((NP + 1, D, PW), BF16),
                        vmem((NP + 1, PW, D), BF16), vmem((NP + 1, PW, D), BF16),
                        vmem((B, SQ, D), F32), vmem((B, SQ, D), F32),
                        vmem((4, SQ, 128), BF16), vmem((4, SQ, 128), BF16),
                        vmem((2, SQ, SK), F32), vmem((2, SQ, SK), F32),
                        vmem((2, 8, SQ, 128), BF16), vmem((2, 8, SQ, 128), BF16),
                        vmem((2, SQ, 128), F32), vmem((2, SQ, 128), F32),
                        vmem((2, PW, 128), BF16), vmem((2, PW, 128), BF16),
                        vmem((3, SQ, 128), BF16), vmem((3, SQ, 128), BF16),
                        vmem((B, SQ, 2 * D), BF16),
                        dma((2 * R + 12,)), dma((14,)), dma((B + 1,))],
        compiler_params=pltpu.CompilerParams(vmem_limit_bytes=110 * 1024 * 1024),
    )(A_x, tr(A_k_cache), tr(A_v_cache), A_wq, A_wo, B_x, tr(B_k_cache), tr(B_v_cache), B_wq, B_wo)
```

```python
import numpy as np
import jax
import jax.numpy as jnp
from jax import lax
import jax.experimental.pallas as pl
import jax.experimental.pallas.tpu as pltpu

B, SQ, D = 8, 240, 640
H, SK, DH = 32, 1024, 192
PW = 2 * DH
NP = H // 2
T = NP * B
U = 2
T1 = 2
RG = 16
QT = ((0, 128), (128, SQ))
LOG2E = 1.4426950408889634
F32, BF16 = jnp.float32, jnp.bfloat16
NT = (((1,), (1,)), ((), ()))

ORDER_FINE = 'q0-q1-q2-k00-k01-k02-k03-k04-k05-k06-k07-k10-k11-k12-k13-k14-k15-k16-k17-P00-P01-P10-t0-P11-t1-o0-o1-o2-o3-o4'
ORDER_U1 = 'q0-q1-q2-k00-k01-k02-k03-k04-k05-k06-k07-k10-k11-P00-P01-P10-t0-P11-t1-k12-k13-k14-k15-k16-o0-o1-o2-o3-o4-k17'
ORDER_LAST = ORDER_U1
ORD4 = [
    'q0-q1-q2-k00-k03-k05-k10-k04-k07-k02-k11-P00-P01-k06-P10-k15-t0-k01-P11-k13-k14-k12-t1-k16-o1-o2-o3-o0-o4-k17',
    'q0-q1-q2-k03-k04-k00-k05-k07-k10-k06-k01-k02-k11-P01-P00-P10-k15-t0-P11-k12-k13-t1-k14-k16-o1-o2-o0-o4-k17-o3',
    'q0-q1-q2-k00-k03-k07-k05-k10-k04-k02-P00-P01-k06-k01-k11-P10-k15-P11-t0-k12-k13-k14-t1-k16-o1-o2-k17-o3-o4-o0',
    'q0-q1-q2-k02-k00-k01-k04-k03-k05-k06-P01-k07-k11-P00-k10-P10-t0-P11-t1-k12-k13-k14-k16-o0-o1-k15-o4-o3-o2-k17',
]
HOOK = 6
HOOK1 = 3


def _qk_tasks(x_ref, wq_ref, kt_ref, q_scr, s_scr):
    c = np.float32(DH ** -0.5 * LOG2E)

    def qproj(n):
        def f():
            q = jnp.dot(x_ref[...], wq_ref[:, n * 128:(n + 1) * 128], preferred_element_type=F32) * c
            if n == 0:
                q_scr[0] = q.astype(BF16)
            elif n == 2:
                q_scr[3] = q.astype(BF16)
            else:
                lane = lax.broadcasted_iota(jnp.int32, (SQ, 128), 1)
                q_scr[1] = jnp.where(lane < 64, q, 0.0).astype(BF16)
                q_scr[2] = jnp.where(lane >= 64, q, 0.0).astype(BF16)
        return f

    def qk(hh, n):
        def f():
            qq = jnp.concatenate([q_scr[2 * hh], q_scr[2 * hh + 1]], axis=1)
            s_scr[hh, :, n * 128:(n + 1) * 128] = jnp.dot(
                qq, kt_ref[hh * 128:hh * 128 + 256, n * 128:(n + 1) * 128], preferred_element_type=F32)
        return f

    tasks = {'q%d' % n: qproj(n) for n in range(3)}
    tasks.update({'k%d%d' % (hh, n): qk(hh, n) for hh in range(2) for n in range(8)})
    return tasks


def _softmax(s_scr, p_scr, l_scr):
    for hh in range(2):
        for r in range(SQ // RG):
            rows = slice(r * RG, (r + 1) * RG)
            s = s_scr[hh, rows, :]
            m = jnp.broadcast_to(jnp.max(s, axis=-1, keepdims=True), (RG, 128))
            acc = None
            for n in range(8):
                e = jnp.exp2(s[:, n * 128:(n + 1) * 128] - m)
                p_scr[hh, n, rows, :] = e.astype(BF16)
                acc = e if acc is None else acc + e
            l_scr[hh, rows, :] = acc


def _pv_tasks(vt_ref, wo_ref, p_scr, l_scr, ot_scr, o_scr, acc_ref, st_ref):
    def pv(hh, qt):
        lo, hi = QT[qt]

        def f():
            p = jnp.concatenate([p_scr[hh, n, lo:hi, :] for n in range(8)], axis=1)
            ot = lax.dot_general(vt_ref[hh * DH:(hh + 1) * DH, :], p, NT, preferred_element_type=F32)
            l = jnp.sum(l_scr[hh, lo:hi, :].T, axis=0, keepdims=True)
            ot_scr[qt, hh * DH:(hh + 1) * DH, 0:hi - lo] = (ot * (1.0 / l)).astype(BF16)
        return f

    def tr(qt):
        lo, hi = QT[qt]

        def f():
            for kt in range(3):
                o_scr[kt, lo:hi, :] = ot_scr[qt, kt * 128:(kt + 1) * 128, 0:hi - lo].T
        return f

    def outp(n):
        def f():
            cols = slice(n * 128, (n + 1) * 128)
            o = jnp.concatenate([o_scr[0], o_scr[1], o_scr[2]], axis=1)
            new = acc_ref[:, cols] + jnp.dot(o, wo_ref[:, cols], preferred_element_type=F32)
            acc_ref[:, cols] = new
            st_ref[:, cols] = new.astype(BF16)
        return f

    tasks = {'P%d%d' % (hh, qt): pv(hh, qt) for hh in range(2) for qt in range(2)}
    tasks.update({'t%d' % qt: tr(qt) for qt in range(2)})
    tasks.update({'o%d' % n: outp(n) for n in range(5)})
    return tasks


def _sub(order, qk_args, sm_args, pv_args, pre=None, hook=None, hook_pos=0):
    pre = dict(pre or {})
    tasks = {}
    if qk_args:
        tasks.update(_qk_tasks(*qk_args))
    if pv_args:
        tasks.update(_pv_tasks(*pv_args))
    if 'q' in pre:
        pre.pop('q')()
    if sm_args:
        _softmax(*sm_args)
    idx = 0
    for name in order.split('-'):
        if name not in tasks:
            continue
        if hook is not None and idx == hook_pos:
            hook()
            hook = None
        if name[0] in pre:
            pre.pop(name[0])()
        tasks[name]()
        idx += 1
    assert hook is None and not pre


def _kernel(xa_h, kta_h, vta_h, wqa_h, woa_h, xb_h, ktb_h, vtb_h, wqb_h, wob_h, out_h,
            xr, kvr, wqa, wqb, woa, wob, acc_a, acc_b,
            qa, qb, sa, sb, pa, pb, la, lb, ota, otb, oa, ob, ostage,
            sem, sem_p, sem_o):
    XB, XA, KB, VA, KA, VB = 0, 1, 0, 1, 2, 3
    R = 2 * U

    def slot(t):
        return (t + 1) & (R - 1)

    def kv_src(h, t):
        tc = jnp.minimum(t, T - 1)
        return h.at[tc & 7, pl.ds(pl.multiple_of((tc >> 3) * PW, 128), PW), :]

    def w_region(dst, c, n, is_q):
        g1 = jnp.minimum((c >> 3) + 1, NP)
        if is_q:
            return dst.at[g1, pl.ds(pl.multiple_of((c & 7) * 80, 16), 80 * n), :]
        return dst.at[g1, pl.ds(pl.multiple_of((c & 7) * 48, 16), 48 * n), :]

    def w_src(h, c, is_q):
        gc = jnp.minimum((c >> 3) + 1, NP - 1)
        if is_q:
            return h.at[pl.ds(pl.multiple_of((c & 7) * 80, 16), 80), pl.ds(pl.multiple_of(gc * PW, 128), PW)]
        return h.at[pl.ds(pl.multiple_of(gc * PW + (c & 7) * 48, 16), 48), :]

    def blocks(t, steady):
        sl = slot(t)

        def cp(src, dst, half, kind):
            fine, coarse = sl * 2 + half, 2 * R + (sl // U) * 6 + kind
            idx = coarse if steady else jnp.where(t <= T1, fine, coarse)
            return pltpu.make_async_copy(src, dst, sem.at[idx])
        return ([cp(xb_h.at[t & 7], xr.at[sl, XB], 0, 1),
                 cp(kv_src(ktb_h, t), kvr.at[sl, KB], 0, 0),
                 cp(kv_src(vta_h, t), kvr.at[sl, VA], 0, 0),
                 cp(w_src(wqb_h, t + 1, True), w_region(wqb, t + 1, 1, True), 0, 3),
                 cp(w_src(woa_h, t + 1, False), w_region(woa, t + 1, 1, False), 0, 4)],
                [cp(xa_h.at[(t + 1) & 7], xr.at[sl, XA], 1, 1),
                 cp(kv_src(kta_h, t + 1), kvr.at[sl, KA], 1, 0),
                 cp(kv_src(vtb_h, t), kvr.at[sl, VB], 1, 0),
                 cp(w_src(wqa_h, t + 1, True), w_region(wqa, t + 1, 1, True), 1, 2),
                 cp(w_src(wob_h, t + 1, False), w_region(wob, t + 1, 1, False), 1, 5)])

    def start_blocks(t, steady):
        h0, h1 = blocks(t, steady)
        for c in h0 + h1:
            c.start()

    def wait_group(t):
        s0 = pl.multiple_of(slot(t), U)
        base = 2 * R + (s0 // U) * 6
        for kind, region in enumerate((kvr.at[pl.ds(s0, U)], xr.at[pl.ds(s0, U)],
                                       w_region(wqa, t + 1, U, True), w_region(wqb, t + 1, U, True),
                                       w_region(woa, t + 1, U, False), w_region(wob, t + 1, U, False))):
            pltpu.make_async_copy(region, region, sem.at[base + kind]).wait()

    def out_copy(b):
        return pltpu.make_async_copy(ostage.at[b], out_h.at[b], sem_o.at[b])

    def body(j, order1, order2, pre1=None, pre2=None, hook=None, hook_pos=0, last=False, mid=None):
        g, b = j >> 3, j & 7
        gn = (j + 1) >> 3
        sl = slot(j)
        _sub(order1, (xr.at[sl, XB], wqb.at[g], kvr.at[sl, KB], qb, sb), (sa, pa, la),
             (kvr.at[sl, VA], woa.at[g], pa, la, ota, oa, acc_a.at[b], ostage.at[b, :, pl.ds(0, D)]),
             pre1, hook, hook_pos)
        if mid is not None:
            mid()
        _sub(order2, None if last else (xr.at[sl, XA], wqa.at[gn], kvr.at[sl, KA], qa, sa), (sb, pb, lb),
             (kvr.at[sl, VB], wob.at[g], pb, lb, otb, ob, acc_b.at[b], ostage.at[b, :, pl.ds(D, D)]),
             pre2)

    n_p = [0]

    def pc(src, dst):
        n_p[0] += 1
        return pltpu.make_async_copy(src, dst, sem_p.at[n_p[0] - 1])
    first = pl.ds(0, PW)
    p_xa0, p_wqa, p_ka0 = pc(xa_h.at[0], xr.at[0, XA]), pc(wqa_h.at[:, first], wqa.at[0]), pc(kta_h.at[0, first, :], kvr.at[0, KA])
    p_xb0, p_wqb, p_kb0 = pc(xb_h.at[0], xr.at[1, XB]), pc(wqb_h.at[:, first], wqb.at[0]), pc(ktb_h.at[0, first, :], kvr.at[1, KB])
    p_va0, p_woa = pc(vta_h.at[0, first, :], kvr.at[1, VA]), pc(woa_h.at[first, :], woa.at[0])
    p_xa1, p_ka1 = pc(xa_h.at[1], xr.at[1, XA]), pc(kta_h.at[1, first, :], kvr.at[1, KA])
    p_vb0, p_wob = pc(vtb_h.at[0, first, :], kvr.at[1, VB]), pc(wob_h.at[first, :], wob.at[0])
    p_wc = []
    for c in range(2):
        p_wc += [pc(w_src(wqa_h, c, True), w_region(wqa, c, 1, True)), pc(w_src(wqb_h, c, True), w_region(wqb, c, 1, True)),
                 pc(w_src(woa_h, c, False), w_region(woa, c, 1, False)), pc(w_src(wob_h, c, False), w_region(wob, c, 1, False))]
    for c in [p_xa0, p_wqa, p_ka0, p_xb0, p_wqb, p_kb0, p_va0, p_woa, p_xa1, p_ka1, p_vb0, p_wob] + p_wc:
        c.start()
    for t in range(1, U):
        start_blocks(t, False)
    acc_a[...] = jnp.zeros(acc_a.shape, F32)
    acc_b[...] = jnp.zeros(acc_b.shape, F32)

    def waits(*cs):
        def f():
            for c in cs:
                c.wait()
        return f

    _sub(ORDER_FINE, (xr.at[0, XA], wqa.at[0], kvr.at[0, KA], qa, sa), None, None,
         {'q': waits(p_xa0, p_wqa), 'k': waits(p_ka0)})
    body(0, ORDER_FINE, ORDER_FINE,
         {'q': waits(p_xb0, p_wqb), 'k': waits(p_kb0), 'P': waits(p_va0, p_woa)},
         {'q': waits(p_xa1, p_ka1), 'P': waits(p_vb0, p_wob)},
         lambda: start_blocks(U, False), HOOK1)
    for c in p_wc:
        c.wait()

    def body1(j, carry):
        h0, h1 = blocks(j, False)
        body(j, ORDER_U1, ORDER_U1, {'q': waits(*h0)}, {'q': waits(*h1)},
             lambda: start_blocks(j + U, False), HOOK1)
        return carry
    lax.fori_loop(1, T1 + 1, body1, 0)

    def body2(i, carry):
        j = T1 + 1 + U * i

        def start_next():
            for k in range(U):
                start_blocks(j + U + k, True)
        wait_group(j)
        for k in range(U):
            body(j + k, ORD4[2 * k], ORD4[2 * k + 1], hook=start_next if k == 0 else None, hook_pos=HOOK)
            pl.when(j + k >= T - B)(lambda: out_copy((j + k) & 7).start())
        return carry
    assert (T1 + 2) % U == 0
    lax.fori_loop(0, (T - 2 - T1) // U, body2, 0)

    wait_group(T - 1)
    out_a = pltpu.make_async_copy(ostage.at[B - 1, :, pl.ds(0, D)], out_h.at[B - 1, :, pl.ds(0, D)], sem_o.at[B - 1])
    out_b = pltpu.make_async_copy(ostage.at[B - 1, :, pl.ds(D, D)], out_h.at[B - 1, :, pl.ds(D, D)], sem_o.at[B])
    body(T - 1, ORDER_LAST, ORDER_LAST, last=True, mid=lambda: out_a.start())
    out_b.start()
    for b in range(B - 1):
        out_copy(b).wait()
    out_a.wait()
    out_b.wait()


@jax.jit
def pallas_concat_heads__gqa_block_cached__gqa_block_cached__near_ridge_kernel(
        A_x, A_k_cache, A_v_cache, A_wq, A_wo, B_x, B_k_cache, B_v_cache, B_wq, B_wo):
    def tr(c):
        return jnp.swapaxes(c, 2, 3).reshape(B, H * DH, SK)
    anyspec = pl.BlockSpec(memory_space=pl.ANY)
    vmem, dma = pltpu.VMEM, pltpu.SemaphoreType.DMA
    R = 2 * U
    return pl.pallas_call(
        _kernel,
        in_specs=[anyspec] * 10,
        out_specs=anyspec,
        out_shape=jax.ShapeDtypeStruct((B, SQ, 2 * D), BF16),
        scratch_shapes=[vmem((R, 2, SQ, D), BF16), vmem((R, 4, PW, SK), BF16),
                        vmem((NP + 1, D, PW), BF16), vmem((NP + 1, D, PW), BF16),
                        vmem((NP + 1, PW, D), BF16), vmem((NP + 1, PW, D), BF16),
                        vmem((B, SQ, D), F32), vmem((B, SQ, D), F32),
                        vmem((4, SQ, 128), BF16), vmem((4, SQ, 128), BF16),
                        vmem((2, SQ, SK), F32), vmem((2, SQ, SK), F32),
                        vmem((2, 8, SQ, 128), BF16), vmem((2, 8, SQ, 128), BF16),
                        vmem((2, SQ, 128), F32), vmem((2, SQ, 128), F32),
                        vmem((2, PW, 128), BF16), vmem((2, PW, 128), BF16),
                        vmem((3, SQ, 128), BF16), vmem((3, SQ, 128), BF16),
                        vmem((B, SQ, 2 * D), BF16),
                        dma((2 * R + 12,)), dma((20,)), dma((B + 1,))],
        compiler_params=pltpu.CompilerParams(vmem_limit_bytes=110 * 1024 * 1024),
    )(A_x, tr(A_k_cache), tr(A_v_cache), A_wq, A_wo, B_x, tr(B_k_cache), tr(B_v_cache), B_wq, B_wo)
```
